```python
import os as _os
_os.environ.setdefault("JAX_PLATFORMS", "cpu")
import jax
import jax.numpy as jnp

def _softmax(x, axis=-1):
    return jax.nn.softmax(x, axis=axis)
def _gelu(x):
    return jax.nn.gelu(x, approximate=True)
def _silu(x):
    return jax.nn.silu(x)
def _sigmoid(x):
    return jax.nn.sigmoid(x)
def _layernorm(x, axis=-1, eps=1e-5):
    m = jnp.mean(x, axis=axis, keepdims=True)
    v = jnp.var(x, axis=axis, keepdims=True)
    return (x - m) / jnp.sqrt(v + eps)
def _scatter_add(tgt, idx, src, axis=0):
    return tgt.at[idx].add(src)
def _segment_sum(src, seg, n):
    return jax.ops.segment_sum(src, seg, n)
class _Rng:
    def __init__(self, key):
        self._k = key
    def _next(self):
        self._k, sub = jax.random.split(self._k)
        return sub
    def normal(self, shape):
        return jax.random.normal(self._next(), shape, dtype=jnp.bfloat16)
    def randint(self, lo, hi, shape):
        return jax.random.randint(self._next(), shape, lo, hi, dtype=jnp.int32)
    def uniform(self, shape, lo=0.0, hi=1.0):
        return jax.random.uniform(self._next(), shape, jnp.bfloat16, lo, hi)
    def permutation(self, n):
        return jax.random.permutation(self._next(), n)


kernel_name = 'concat_heads__gqa_block_cached__sliding_block_cached__decode'

def setup_inputs():
    _rng = _Rng(jax.random.key(int.from_bytes(__import__("os").urandom(4), "little")))
    _w = (lambda a: (lambda t: t.astype(jnp.bfloat16) if jnp.issubdtype(t.dtype, jnp.floating) else t)(jnp.asarray(a)))
    def _A_setup():
        B, Sq, D = 2, 1, 448
        Hq, Hkv, Sk, Dh = 16, 8, 8192, 256
        assert Hq % Hkv == 0, (Hq, Hkv)
        return {
            "x": _w((lambda *s: _rng.normal(s) * 0.8)(B, Sq, D)),
            "k_cache": _w((lambda *s: _rng.normal(s) * 0.8)(B, Hkv, Sk, Dh)),
            "v_cache": _w((lambda *s: _rng.normal(s) * 0.05)(B, Hkv, Sk, Dh)),
            "wq": _w((lambda *s: _rng.normal(s) * 0.8)(D, Hq * Dh) * (D ** -0.5)),
            "wo": _w((lambda *s: _rng.normal(s) * 0.05)(Hq * Dh, D) * ((Hq * Dh) ** -0.5)),
        }
    _A_in = _A_setup()

    def _B_setup():
        B, Sq, D = 2, 1, 448
        Hq, Hkv, Sk, Dh = 16, 8, 8192, 256
        assert Hq % Hkv == 0, (Hq, Hkv)
        return {
            "x": _w((lambda *s: _rng.normal(s) * 0.8)(B, Sq, D)),
            "k_cache": _w((lambda *s: _rng.normal(s) * 0.8)(B, Hkv, Sk, Dh)),
            "v_cache": _w((lambda *s: _rng.normal(s) * 0.05)(B, Hkv, Sk, Dh)),
            "wq": _w((lambda *s: _rng.normal(s) * 0.8)(D, Hq * Dh) * (D ** -0.5)),
            "wo": _w((lambda *s: _rng.normal(s) * 0.05)(Hq * Dh, D) * ((Hq * Dh) ** -0.5)),
        }
    _B_in = _B_setup()

    return {
        "A_x": _A_in["x"],
        "A_k_cache": _A_in["k_cache"],
        "A_v_cache": _A_in["v_cache"],
        "A_wq": _A_in["wq"],
        "A_wo": _A_in["wo"],
        "B_x": _B_in["x"],
        "B_k_cache": _B_in["k_cache"],
        "B_v_cache": _B_in["v_cache"],
        "B_wq": _B_in["wq"],
        "B_wo": _B_in["wo"],
    }

def reference(A_x, A_k_cache, A_v_cache, A_wq, A_wo, B_x, B_k_cache, B_v_cache, B_wq, B_wo):
    def _A_ref(x, k_cache, v_cache, wq, wo):
        B, Sq, D = x.shape
        Hq, Dh = 16, 256
        Hkv = k_cache.shape[1]
        rep = Hq // Hkv
        q = (lambda x, *d: x.transpose(*d))((x @ wq).reshape(B, Sq, Hq, Dh), 0, 2, 1, 3)
        k = jnp.repeat(k_cache, rep, axis=1)
        v = jnp.repeat(v_cache, rep, axis=1)
        scores = jnp.einsum("bhqd,bhkd->bhqk", q, k) * (Dh ** -0.5)
        p = _softmax(scores, axis=-1)
        o = jnp.einsum("bhqk,bhkd->bhqd", p, v)
        return (lambda x, *d: x.transpose(*d))(o, 0, 2, 1, 3).reshape(B, Sq, Hq * Dh) @ wo

    def _B_ref(x, k_cache, v_cache, wq, wo):
        B, Sq, D = x.shape
        Hq, Dh = 16, 256
        Hkv, Sk = k_cache.shape[1], k_cache.shape[2]
        W = min(4096, max(256, Sk // 4))
        rep = Hq // Hkv
        q = (lambda x, *d: x.transpose(*d))((x @ wq).reshape(B, Sq, Hq, Dh), 0, 2, 1, 3)
        k = jnp.repeat(k_cache[:, :, Sk - W:, :], rep, axis=1)
        v = jnp.repeat(v_cache[:, :, Sk - W:, :], rep, axis=1)
        scores = jnp.einsum("bhqd,bhkd->bhqk", q, k) * (Dh ** -0.5)
        p = _softmax(scores, axis=-1)
        o = jnp.einsum("bhqk,bhkd->bhqd", p, v)
        return (lambda x, *d: x.transpose(*d))(o, 0, 2, 1, 3).reshape(B, Sq, Hq * Dh) @ wo

    a = _A_ref(A_x, A_k_cache, A_v_cache, A_wq, A_wo)
    b = _B_ref(B_x, B_k_cache, B_v_cache, B_wq, B_wo)
    return jnp.concatenate([a, b], axis=-1)
```

```python
import jax
import jax.numpy as jnp
from jax import lax
import jax.experimental.pallas as pl
import jax.experimental.pallas.tpu as pltpu

HQ = 16
DH = 256
KEYS = 128
DMA_ROWS = 64
SLOTS = 8
W_ROWS = 8
W_COLS = 2048

_NT = (((1,), (1,)), ((), ()))


def _kernel(xa_hbm, ka_hbm, va_hbm, wqa_hbm, woa_hbm,
            xb_hbm, kb_hbm, vb_hbm, wqb_hbm, wob_hbm,
            out_ref,
            x_buf, wq_buf, wo_buf, kv_buf, x_sem, wq_sem, wo_sem, kv_sem,
            *, window):
    nb, hkv, sk, _ = ka_hbm.shape
    d_model = xa_hbm.shape[1]
    rep = HQ // hkv
    steps_a = sk // KEYS
    steps_b = window // KEYS
    start_b = kb_hbm.shape[2] - window
    total_a = nb * steps_a
    total = total_a + nb * steps_b

    def start_kv(k_hbm, v_hbm, b, row0, slot):
        n = 0
        for which, src in enumerate((k_hbm, v_hbm)):
            for c in range(KEYS // DMA_ROWS):
                for h in range(hkv):
                    pltpu.make_async_copy(
                        src.at[b, h, pl.ds(row0 + c * DMA_ROWS, DMA_ROWS), :],
                        kv_buf.at[slot, which, pl.ds(h * KEYS + c * DMA_ROWS, DMA_ROWS), :],
                        kv_sem.at[slot],
                    ).start(priority=n % 2)
                    n += 1

    def start_step(g):
        slot = g % SLOTS

        def start_a():
            start_kv(ka_hbm, va_hbm, g // steps_a,
                     pl.multiple_of((g % steps_a) * KEYS, KEYS), slot)

        def start_b_():
            gb = g - total_a
            start_kv(kb_hbm, vb_hbm, gb // steps_b,
                     pl.multiple_of(start_b + (gb % steps_b) * KEYS, DMA_ROWS), slot)

        if isinstance(g, int):
            start_a() if g < total_a else start_b_()
        else:
            pl.when(g < total_a)(start_a)
            pl.when(jnp.logical_and(g >= total_a, g < total))(start_b_)

    def wait_step(slot):
        pltpu.make_async_copy(kv_buf.at[slot], kv_buf.at[slot], kv_sem.at[slot]).wait()

    def start_weights(pairs, sem):
        rows, cols = pairs[0][0].shape
        n_row = rows // W_ROWS
        stride = 8
        n = 0
        for c in range(cols // W_COLS):
            for i in range(stride):
                for r in range(i, n_row, stride):
                    for src, dst in pairs:
                        sl = (pl.ds(r * W_ROWS, W_ROWS), pl.ds(c * W_COLS, W_COLS))
                        pltpu.make_async_copy(src.at[sl], dst.at[sl], sem).start(priority=n % 2)
                        n += 1

    x_copies = [pltpu.make_async_copy(src, x_buf.at[i], x_sem.at[i])
                for i, src in enumerate((xa_hbm, xb_hbm))]
    start_weights([(wqa_hbm, wq_buf.at[0]), (wqb_hbm, wq_buf.at[1])], wq_sem)
    for cp in x_copies:
        cp.start()
    for g in range(SLOTS - 1):
        start_step(g)
    start_weights([(woa_hbm, wo_buf.at[pl.ds(0, d_model)]),
                   (wob_hbm, wo_buf.at[pl.ds(d_model, d_model)])], wo_sem)

    row = lax.broadcasted_iota(jnp.int32, (HQ, 128), 0)
    row_kv = row // rep
    row_q = lax.broadcasted_iota(jnp.int32, (HQ, DH), 0)

    for cp in x_copies:
        cp.wait()
    pltpu.make_async_copy(wq_buf, wq_buf, wq_sem).wait()

    def project_q(i):
        x = x_buf[i].astype(jnp.float32)
        xr = jnp.concatenate(
            [jnp.broadcast_to(x[b:b + 1], (HQ, d_model)) for b in range(nb)], axis=0
        ).astype(jnp.bfloat16)
        qs = [jnp.zeros((HQ, DH), jnp.float32) for _ in range(nb)]
        for h in range(HQ):
            full = jnp.dot(xr, wq_buf[i, :, h * DH:(h + 1) * DH],
                           preferred_element_type=jnp.float32)
            for b in range(nb):
                qs[b] = jnp.where(row_q == h, full[b * HQ:(b + 1) * HQ], qs[b])
        return [q.astype(jnp.bfloat16) for q in qs]

    q_all = project_q(0) + project_q(1)

    scale = DH ** -0.5

    def attend(q, g0, n_steps):
        def body(j, carry):
            m, l, acc = carry
            g = g0 + j
            slot = g % SLOTS
            wait_step(slot)
            start_step(g + SLOTS - 1)
            s_all = lax.dot_general(q, kv_buf[slot, 0], _NT,
                                    preferred_element_type=jnp.float32)
            s = s_all[:, :KEYS]
            for h in range(1, hkv):
                s = jnp.where(row_kv == h, s_all[:, h * KEYS:(h + 1) * KEYS], s)
            s = s * scale
            m_new = jnp.maximum(m, jnp.max(s, axis=1, keepdims=True))
            alpha = jnp.exp(m - m_new)
            p = jnp.exp(s - m_new)
            l = alpha * l + p
            p_all = jnp.concatenate(
                [jnp.where(row_kv == h, p, 0.0).astype(jnp.bfloat16) for h in range(hkv)],
                axis=1)
            pv = jnp.dot(p_all, kv_buf[slot, 1], preferred_element_type=jnp.float32)
            acc = jnp.concatenate([alpha] * (DH // 128), axis=1) * acc + pv
            return m_new, l, acc

        init = (jnp.full((HQ, 128), -jnp.inf, jnp.float32),
                jnp.zeros((HQ, 128), jnp.float32),
                jnp.zeros((HQ, DH), jnp.float32))
        _, l, acc = lax.fori_loop(0, n_steps, body, init)
        return acc / jnp.sum(l, axis=1, keepdims=True)

    outs = []
    for b in range(nb):
        outs.append(attend(q_all[b], b * steps_a, steps_a))
    for b in range(nb):
        outs.append(attend(q_all[nb + b], total_a + b * steps_b, steps_b))

    lhs = []
    for h in range(HQ):
        blk = jnp.zeros((HQ, DH), jnp.float32)
        for i, o in enumerate(outs):
            blk = jnp.where(row_q == i, jnp.broadcast_to(o[h:h + 1], (HQ, DH)), blk)
        lhs.append(blk.astype(jnp.bfloat16))
    lhs = jnp.concatenate(lhs, axis=1)
    pltpu.make_async_copy(wo_buf, wo_buf, wo_sem).wait()
    res = lax.dot_general(lhs, wo_buf[...], _NT, preferred_element_type=jnp.float32)
    col = lax.broadcasted_iota(jnp.int32, (nb, 2 * d_model), 1)
    out_ref[...] = jnp.where(col < d_model, res[0:nb], res[nb:2 * nb]).astype(out_ref.dtype)


@jax.jit
def pallas_concat_heads__gqa_block_cached__sliding_block_cached__decode_kernel(
    A_x: jax.Array,
    A_k_cache: jax.Array,
    A_v_cache: jax.Array,
    A_wq: jax.Array,
    A_wo: jax.Array,
    B_x: jax.Array,
    B_k_cache: jax.Array,
    B_v_cache: jax.Array,
    B_wq: jax.Array,
    B_wo: jax.Array,
):
    nb, sq, d_model = A_x.shape
    hkv = A_k_cache.shape[1]
    window = min(4096, max(256, B_k_cache.shape[2] // 4))
    assert sq == 1

    hbm = pl.BlockSpec(memory_space=pltpu.HBM)
    out = pl.pallas_call(
        lambda *refs: _kernel(*refs, window=window),
        in_specs=[hbm] * 10,
        out_specs=pl.BlockSpec(memory_space=pltpu.VMEM),
        out_shape=jax.ShapeDtypeStruct((nb, 2 * d_model), A_x.dtype),
        scratch_shapes=[
            pltpu.VMEM((2, nb, d_model), jnp.bfloat16),
            pltpu.VMEM((2, d_model, HQ * DH), jnp.bfloat16),
            pltpu.VMEM((2 * d_model, HQ * DH), jnp.bfloat16),
            pltpu.VMEM((SLOTS, 2, hkv * KEYS, DH), jnp.bfloat16),
            pltpu.SemaphoreType.DMA((2,)),
            pltpu.SemaphoreType.DMA(()),
            pltpu.SemaphoreType.DMA(()),
            pltpu.SemaphoreType.DMA((SLOTS,)),
        ],
        compiler_params=pltpu.CompilerParams(vmem_limit_bytes=64 * 1024 * 1024),
    )(A_x.reshape(nb, d_model), A_k_cache, A_v_cache, A_wq, A_wo.T,
      B_x.reshape(nb, d_model), B_k_cache, B_v_cache, B_wq, B_wo.T)
    return out.reshape(nb, sq, 2 * d_model)
```

```python
import functools
import itertools

import jax
import jax.numpy as jnp
from jax import lax
import jax.experimental.pallas as pl
import jax.experimental.pallas.tpu as pltpu

HQ = 16
DH = 256
LANES = 128
KEYS = 128
KV_ROWS = 64
W_COLS = 2048
W_ROWS = 8
W_BAND = 64
SLOTS = 5

_NT = (((1,), (1,)), ((), ()))
_F32, _BF16 = jnp.float32, jnp.bfloat16


def _in_range(i, start, size):
    return jnp.logical_and(i >= start, i < start + size)


def _wait(dst, sem):
    pltpu.make_async_copy(dst, dst, sem).wait()


def _start_weights(src, dst, sem):
    order = itertools.product(range(0, W_BAND, W_ROWS), range(0, dst.shape[0], W_BAND))
    for n, (row, band) in enumerate(order):
        rows = pl.ds(band + row, W_ROWS)
        pltpu.make_async_copy(src.at[rows, :], dst.at[rows, :], sem).start(priority=n % 2)


def _start_kv(k_hbm, v_hbm, b, key0, dst, sem):
    half = k_hbm.shape[1] // 2
    order = itertools.product(range(0, KEYS, KV_ROWS), range(half), range(2), range(2))
    for row, h, upper, kv in order:
        head = upper * half + h
        pltpu.make_async_copy(
            (k_hbm, v_hbm)[kv].at[b, head, pl.ds(key0 + row, KV_ROWS), :],
            dst.at[kv, pl.ds(head * KEYS + row, KV_ROWS), :],
            sem,
        ).start(priority=kv)


def _kernel(xa_hbm, ka_hbm, va_hbm, wqa_hbm, woa_hbm,
            xb_hbm, kb_hbm, vb_hbm, wqb_hbm, wob_hbm,
            out_ref,
            x_buf,
            wq_buf,
            wo_buf,
            kv_buf,
            q_buf,
            o_buf,
            res_buf,
            m_ref, l_ref, acc_ref,
            x_sem, ring_sems, tail_sems,
            *, window):
    nb, hkv, sk, _ = ka_hbm.shape
    d_model = xa_hbm.shape[1]
    d_pad = wo_buf.shape[1]
    shift = d_pad - d_model
    steps_a = sk // KEYS
    steps_b = window // KEYS
    first_key_b = kb_hbm.shape[2] - window
    ahead = SLOTS - 1
    parts = HQ * DH // W_COLS
    pieces = tail_sems.shape[0]

    j_kva = 2 * parts
    j_woa = j_kva + nb * steps_a
    j_kvb = j_woa + parts
    j_wob = j_kvb + nb * steps_b

    x_copies = [pltpu.make_async_copy(src, x_buf.at[i], x_sem)
                for i, src in enumerate((xa_hbm, xb_hbm))]

    def cols(c):
        return pl.ds(pl.multiple_of(c * W_COLS, W_COLS), W_COLS)

    def for_piece(p, fn):
        tile, c = lax.div(p, parts), lax.rem(p, parts)

        @pl.when(tile == 0)
        def _():
            fn(wob_hbm.at[pl.ds(0, LANES - shift), cols(c)],
               wo_buf.at[1, pl.ds(shift, LANES - shift), cols(c)], tail_sems.at[p])

        @pl.when(tile > 0)
        def _():
            fn(wob_hbm.at[pl.ds(pl.multiple_of(tile * LANES - shift, shift), LANES), cols(c)],
               wo_buf.at[1, pl.ds(pl.multiple_of(tile * LANES, LANES), LANES), cols(c)],
               tail_sems.at[p])

    def start_job(r):
        slot = lax.rem(r, SLOTS)
        sem = ring_sems.at[slot]

        @pl.when(r < parts)
        def _():
            _start_weights(wqa_hbm.at[:, cols(r)], wq_buf.at[0, :, cols(r)], sem)

        @pl.when(r == 0)
        def _():
            for copy in x_copies:
                copy.start()

        @pl.when(_in_range(r, parts, parts))
        def _():
            _start_weights(wqb_hbm.at[:, cols(r - parts)], wq_buf.at[1, :, cols(r - parts)], sem)

        @pl.when(_in_range(r, j_kva, nb * steps_a))
        def _():
            g = r - j_kva
            key0 = pl.multiple_of(lax.rem(g, steps_a) * KEYS, KEYS)
            _start_kv(ka_hbm, va_hbm, lax.div(g, steps_a), key0, kv_buf.at[slot], sem)

        @pl.when(_in_range(r, j_woa, parts))
        def _():
            _start_weights(woa_hbm.at[:, cols(r - j_woa)],
                           wo_buf.at[0, pl.ds(0, d_model), cols(r - j_woa)], sem)

        @pl.when(_in_range(r, j_kvb, nb * steps_b))
        def _():
            g = r - j_kvb
            key0 = pl.multiple_of(first_key_b + lax.rem(g, steps_b) * KEYS, KEYS)
            _start_kv(kb_hbm, vb_hbm, lax.div(g, steps_b), key0, kv_buf.at[slot], sem)

        @pl.when(r >= j_wob)
        def _():
            @pl.loop(0, pieces // ahead)
            def _(k):
                for_piece((r - j_wob) * (pieces // ahead) + k, _start_weights)

    def init():
        q_buf[...] = jnp.zeros(q_buf.shape, _F32)
        o_buf[...] = jnp.zeros(o_buf.shape, _F32)
        res_buf[...] = jnp.zeros(res_buf.shape, _F32)

        @pl.loop(0, HQ)
        def _(h):
            head = pl.ds(pl.multiple_of(h * DH, DH), DH)
            wo_buf[0, d_model:, head] = jnp.zeros((shift, DH), _BF16)
            wo_buf[1, :shift, head] = jnp.zeros((shift, DH), _BF16)

        for copy in x_copies:
            copy.wait()

    q_row = lax.broadcasted_iota(jnp.int32, (HQ, DH), 0)
    kv_of_row = lax.broadcasted_iota(jnp.int32, (HQ, KEYS), 0) // (HQ // hkv)

    def project_q(r):
        branch, c = lax.div(r, parts), lax.rem(r, parts)
        _wait(wq_buf.at[branch, :, cols(c)], ring_sems.at[lax.rem(r, SLOTS)])
        x = x_buf[branch].astype(_F32)
        x = jnp.concatenate([jnp.broadcast_to(x[b:b + 1], (HQ, d_model)) for b in range(nb)],
                            axis=0).astype(_BF16)

        @pl.loop(0, W_COLS // (2 * DH))
        def _(pair):
            h0 = c * (W_COLS // DH) + 2 * pair
            w = wq_buf[branch, :, pl.ds(pl.multiple_of(h0 * DH, 2 * DH), 2 * DH)]
            full = jnp.dot(x, w, preferred_element_type=_F32)
            for b in range(nb):
                q = q_buf[branch, b]
                for u in range(2):
                    q = jnp.where(q_row == h0 + u,
                                  full[b * HQ:(b + 1) * HQ, u * DH:(u + 1) * DH], q)
                q_buf[branch, b] = q

    def attend(r):
        second = r >= j_kvb
        branch = second.astype(jnp.int32)
        g = r - jnp.where(second, j_kvb, j_kva)
        steps = jnp.where(second, steps_b, steps_a)
        b = lax.div(g, steps)
        step = g - b * steps
        slot = lax.rem(r, SLOTS)

        @pl.when(step == 0)
        def _():
            m_ref[...] = jnp.full(m_ref.shape, jnp.finfo(_F32).min, _F32)
            l_ref[...] = jnp.zeros(l_ref.shape, _F32)
            acc_ref[...] = jnp.zeros(acc_ref.shape, _F32)

        _wait(kv_buf.at[slot], ring_sems.at[slot])
        s_all = lax.dot_general(q_buf[branch, b].astype(_BF16), kv_buf[slot, 0], _NT,
                                preferred_element_type=_F32)
        s = s_all[:, :KEYS]
        for h in range(1, hkv):
            s = jnp.where(kv_of_row == h, s_all[:, h * KEYS:(h + 1) * KEYS], s)
        s = s * (DH ** -0.5)
        m_old = m_ref[...]
        m_new = jnp.maximum(m_old, jnp.max(s, axis=1, keepdims=True))
        alpha = jnp.exp(m_old - m_new)
        p = jnp.exp(s - m_new)
        m_ref[...] = m_new
        l_ref[...] = alpha * l_ref[...] + p
        p_all = jnp.concatenate([jnp.where(kv_of_row == h, p, 0.0) for h in range(hkv)], axis=1)
        pv = jnp.dot(p_all.astype(_BF16), kv_buf[slot, 1], preferred_element_type=_F32)
        acc_ref[...] = jnp.concatenate([alpha] * (DH // KEYS), axis=1) * acc_ref[...] + pv

        @pl.when(step == steps - 1)
        def _():
            o = acc_ref[...] / jnp.sum(l_ref[...], axis=1, keepdims=True)
            shape = (o_buf.shape[1], DH)
            mine = lax.broadcasted_iota(jnp.int32, shape, 0) == b
            for h in range(HQ):
                head = slice(h * DH, (h + 1) * DH)
                o_buf[branch, :, head] = jnp.where(
                    mine, jnp.broadcast_to(o[h:h + 1], shape), o_buf[branch, :, head])

    def project_out_a(r):
        c = r - j_woa
        _wait(wo_buf.at[0, pl.ds(0, d_model), cols(c)], ring_sems.at[lax.rem(r, SLOTS)])

        @pl.loop(0, 2)
        def _(u):
            size = W_COLS // 2
            k = pl.ds(pl.multiple_of(c * W_COLS + u * size, size), size)
            res_buf[0] += lax.dot_general(o_buf[0, :, k].astype(_BF16), wo_buf[0, :, k], _NT,
                                          preferred_element_type=_F32)

    @pl.loop(0, j_wob + ahead)
    def _(t):
        start_job(t)
        r = t - ahead
        pl.when(r == -1)(init)
        pl.when(_in_range(r, 0, j_kva))(lambda: project_q(r))
        pl.when(jnp.logical_or(_in_range(r, j_kva, nb * steps_a), r >= j_kvb))(lambda: attend(r))
        pl.when(_in_range(r, j_woa, parts))(lambda: project_out_a(r))

    @pl.loop(0, pieces)
    def _(p):
        k = cols(lax.rem(p, parts))
        tile = pl.ds(pl.multiple_of(lax.div(p, parts) * LANES, LANES), LANES)
        o = o_buf[1, :, k].astype(_BF16)
        for_piece(p, lambda src, dst, sem: _wait(dst, sem))
        res_buf[1, :, tile] += lax.dot_general(o, wo_buf[1, tile, k], _NT,
                                               preferred_element_type=_F32)

    last = d_pad - LANES
    res_a, res_b = res_buf[0, :nb], res_buf[1, :nb]
    from_a = lax.broadcasted_iota(jnp.int32, (nb, LANES), 1) < d_model - last
    shared = jnp.where(from_a, res_a[:, last:], res_b[:, :LANES])
    out_ref[...] = jnp.concatenate(
        [res_a[:, :last], shared, res_b[:, LANES:]], axis=1).astype(out_ref.dtype)


@jax.jit
def pallas_concat_heads__gqa_block_cached__sliding_block_cached__decode_kernel(
    A_x: jax.Array,
    A_k_cache: jax.Array,
    A_v_cache: jax.Array,
    A_wq: jax.Array,
    A_wo: jax.Array,
    B_x: jax.Array,
    B_k_cache: jax.Array,
    B_v_cache: jax.Array,
    B_wq: jax.Array,
    B_wo: jax.Array,
):
    nb, sq, d_model = A_x.shape
    hkv = A_k_cache.shape[1]
    window = min(4096, max(256, B_k_cache.shape[2] // 4))
    d_pad = pl.cdiv(d_model, LANES) * LANES
    pieces = (d_pad // LANES) * (HQ * DH // W_COLS)
    assert sq == 1 and nb <= 8 and d_pad - d_model == LANES // 2 and pieces % (SLOTS - 1) == 0
    assert A_k_cache.shape[2] % KEYS == 0 and B_k_cache.shape[2] % KEYS == 0 and window % KEYS == 0

    out = pl.pallas_call(
        functools.partial(_kernel, window=window),
        in_specs=[pl.BlockSpec(memory_space=pltpu.HBM)] * 10,
        out_specs=pl.BlockSpec(memory_space=pltpu.VMEM),
        out_shape=jax.ShapeDtypeStruct((nb, 2 * d_model), A_x.dtype),
        scratch_shapes=[
            pltpu.VMEM((2, nb, d_model), _BF16),
            pltpu.VMEM((2, d_model, HQ * DH), _BF16),
            pltpu.VMEM((2, d_pad, HQ * DH), _BF16),
            pltpu.VMEM((SLOTS, 2, hkv * KEYS, DH), _BF16),
            pltpu.VMEM((2, nb, HQ, DH), _F32),
            pltpu.VMEM((2, 8, HQ * DH), _F32),
            pltpu.VMEM((2, 8, d_pad), _F32),
            pltpu.VMEM((HQ, KEYS), _F32),
            pltpu.VMEM((HQ, KEYS), _F32),
            pltpu.VMEM((HQ, DH), _F32),
            pltpu.SemaphoreType.DMA(()),
            pltpu.SemaphoreType.DMA((SLOTS,)),
            pltpu.SemaphoreType.DMA((pieces,)),
        ],
        compiler_params=pltpu.CompilerParams(vmem_limit_bytes=48 * 1024 * 1024),
    )(A_x.reshape(nb, d_model), A_k_cache, A_v_cache, A_wq, A_wo.T,
      B_x.reshape(nb, d_model), B_k_cache, B_v_cache, B_wq, B_wo.T)
    return out.reshape(nb, sq, 2 * d_model)
```
